```python
import os as _os
_os.environ.setdefault("JAX_PLATFORMS", "cpu")
import jax
import jax.numpy as jnp

def _softmax(x, axis=-1):
    return jax.nn.softmax(x, axis=axis)
def _gelu(x):
    return jax.nn.gelu(x, approximate=True)
def _silu(x):
    return jax.nn.silu(x)
def _sigmoid(x):
    return jax.nn.sigmoid(x)
def _layernorm(x, axis=-1, eps=1e-5):
    m = jnp.mean(x, axis=axis, keepdims=True)
    v = jnp.var(x, axis=axis, keepdims=True)
    return (x - m) / jnp.sqrt(v + eps)
def _scatter_add(tgt, idx, src, axis=0):
    return tgt.at[idx].add(src)
def _segment_sum(src, seg, n):
    return jax.ops.segment_sum(src, seg, n)
class _Rng:
    def __init__(self, key):
        self._k = key
    def _next(self):
        self._k, sub = jax.random.split(self._k)
        return sub
    def normal(self, shape):
        return jax.random.normal(self._next(), shape, dtype=jnp.bfloat16)
    def randint(self, lo, hi, shape):
        return jax.random.randint(self._next(), shape, lo, hi, dtype=jnp.int32)
    def uniform(self, shape, lo=0.0, hi=1.0):
        return jax.random.uniform(self._next(), shape, jnp.bfloat16, lo, hi)
    def permutation(self, n):
        return jax.random.permutation(self._next(), n)


kernel_name = 'gated_mix__linear_attn_block__glu_gated_swiglu__prompt'

def setup_inputs():
    _rng = _Rng(jax.random.key(int.from_bytes(__import__("os").urandom(4), "little")))
    _w = (lambda a: (lambda t: t.astype(jnp.bfloat16) if jnp.issubdtype(t.dtype, jnp.floating) else t)(jnp.asarray(a)))
    def _A_setup():
        B, S, D = 1, 2048, 1024
        return {
            "x": _w((lambda *s: _rng.normal(s) * 0.05)(B, S, D)),
            "wqkv": _w((lambda *s: _rng.normal(s) * 0.8)(D, 3 * D)),
            "wo": _w((lambda *s: _rng.normal(s) * 0.05)(D, D)),
        }
    _A_in = _A_setup()

    def _B_setup():
        B, S, D, F = 1, 2048, 1024, 3584
        return {
            "x": _w((lambda *s: _rng.normal(s) * 0.05)(B, S, D)),
            "w1": _w((lambda *s: _rng.normal(s) * 1.6)(D, F) * (2.0 / D) ** 0.5),
            "w3": _w((lambda *s: _rng.normal(s) * 1.6)(D, F) * (2.0 / D) ** 0.5),
            "w2": _w((lambda *s: _rng.normal(s) * 1.6)(F, D) * (2.0 / F) ** 0.5),
        }
    _B_in = _B_setup()

    return {
        "A_x": _A_in["x"],
        "A_wqkv": _A_in["wqkv"],
        "A_wo": _A_in["wo"],
        "B_x": _B_in["x"],
        "B_w1": _B_in["w1"],
        "B_w3": _B_in["w3"],
        "B_w2": _B_in["w2"],
        "gate_w": _w((lambda *s: _rng.normal(s) * 0.05)(1024) * 16.0),
    }

def reference(A_x, A_wqkv, A_wo, B_x, B_w1, B_w3, B_w2, gate_w):
    def _A_ref(x, wqkv, wo):
        B, S, D = x.shape
        H = 32; Dh = D // H
        qkv = (lambda x, *d: x.transpose(*d))((x @ wqkv).reshape(B, S, 3, H, Dh), 2, 0, 3, 1, 4)
        q, k, v = qkv[0], qkv[1], qkv[2]
        phi = lambda t: jnp.where(t > 0, t + 1, jnp.exp(t)) + 1e-6
        pq, pk = phi(q), phi(k)
        kv = jnp.einsum("bhsd,bhse->bhde", pk, v)
        z = jnp.einsum("bhsd->bhd", pk)
        num = jnp.einsum("bhqd,bhde->bhqe", pq, kv)
        den = jnp.einsum("bhqd,bhd->bhq", pq, z)[..., None] + 1e-6
        o = num / den
        return (lambda x, *d: x.transpose(*d))(o, 0, 2, 1, 3).reshape(B, S, D) @ wo

    def _B_ref(x, w1, w3, w2):
        gate = jnp.einsum("bsd,df->bsf", x, w1)
        up = jnp.einsum("bsd,df->bsf", x, w3)
        h = _silu(gate) * up
        out = jnp.einsum("bsf,fd->bsd", h, w2)
        return out

    x = A_x
    g = _sigmoid((x * gate_w).sum(-1, keepdims=True))
    a = _A_ref(x, A_wqkv, A_wo)
    b = _B_ref(x, B_w1, B_w3, B_w2)
    return g * a + (1 - g) * b
```

```python
import jax
import jax.numpy as jnp
import jax.experimental.pallas as pl
import jax.experimental.pallas.tpu as pltpu

S = 2048
D = 1024
F = 3584
DH = 32
TM = 512
NC = S // TM
T = 512
NA = D // T
NF = F // T
NG = D // 128

f32 = jnp.float32
bf16 = jnp.bfloat16


def _phi(t):
    return jnp.where(t > 0, t + 1.0, jnp.exp(t)) + 1e-6


def _kernel(x_hbm, gw_ref, wqkv_hbm, wo_hbm, w1_hbm, w3_hbm, w2_hbm,
            o_hbm,
            x_v, wq_v, wk_v, wv_v, wo_v, w1_v, w3_v, w2_v,
            acc_ref, kva_ref, m_ref, zm_ref, g_ref, o_v,
            sem_x, sem_q, sem_k, sem_v, sem_o, sem_1, sem_3, sem_2, sem_out):

    def cp_x(c):
        return pltpu.make_async_copy(x_hbm.at[pl.ds(c * TM, TM), :], x_v.at[c], sem_x.at[c])

    def cp_q():
        return pltpu.make_async_copy(wqkv_hbm.at[:, pl.ds(0, D)], wq_v, sem_q.at[0])

    def cp_k(j):
        return pltpu.make_async_copy(wqkv_hbm.at[:, pl.ds(D + j * T, T)], wk_v.at[j], sem_k.at[j])

    def cp_v(j):
        return pltpu.make_async_copy(wqkv_hbm.at[:, pl.ds(2 * D + j * T, T)], wv_v.at[j], sem_v.at[j])

    def cp_o():
        return pltpu.make_async_copy(wo_hbm, wo_v, sem_o.at[0])

    def cp_1(j):
        return pltpu.make_async_copy(w1_hbm.at[:, pl.ds(j * T, T)], w1_v.at[j], sem_1.at[j])

    def cp_3(j):
        return pltpu.make_async_copy(w3_hbm.at[:, pl.ds(j * T, T)], w3_v.at[j], sem_3.at[j])

    def cp_2(j):
        return pltpu.make_async_copy(w2_hbm.at[pl.ds(j * T, T), :], w2_v.at[j], sem_2.at[j])

    def cp_out(c):
        return pltpu.make_async_copy(o_v.at[c], o_hbm.at[pl.ds(c * TM, TM), :], sem_out.at[c])

    cp_x(0).start()
    cp_k(0).start()
    cp_v(0).start()
    kva_ref[...] = jnp.zeros_like(kva_ref)
    cp_x(0).wait()
    cp_k(0).wait()
    cp_v(0).wait()
    for c in range(1, NC):
        cp_x(c).start()
    for j in range(1, NA):
        cp_k(j).start()
        cp_v(j).start()

    def kv_body(i, carry):
        s = i // NC
        c = i % NC

        @pl.when(jnp.logical_and(s == 0, c > 0))
        def _():
            cp_x(c).wait()

        @pl.when(jnp.logical_and(c == 0, s > 0))
        def _():
            cp_k(s).wait()
            cp_v(s).wait()

        @pl.when(i == 1)
        def _():
            cp_o().start()
            cp_q().start()
            for j in range(NF):
                cp_1(j).start()
                cp_3(j).start()
                cp_2(j).start()

        x = x_v[c]
        k = jnp.dot(x, wk_v[s], preferred_element_type=f32)
        v = jnp.dot(x, wv_v[s], preferred_element_type=f32)
        pk = _phi(k).astype(bf16)
        vb = v.astype(bf16)
        ones = jnp.ones((TM, 128), bf16)
        for j in range(T // 128):
            pkj = pk[:, j * 128:(j + 1) * 128]
            vaug = jnp.concatenate([vb[:, j * 128:(j + 1) * 128], ones], axis=1)
            kva = jax.lax.dot_general(pkj, vaug, (((0,), (0,)), ((), ())),
                                      preferred_element_type=f32)
            kva_ref[s * (T // 128) + j] += kva
        return carry

    jax.lax.fori_loop(0, NA * NC, kv_body, 0)

    cp_o().wait()
    cp_q().wait()
    ri = jax.lax.broadcasted_iota(jnp.int32, (128, 128), 0) // DH
    ci = jax.lax.broadcasted_iota(jnp.int32, (128, 128), 1) // DH
    mask = ri == ci
    for gidx in range(NG):
        kva = kva_ref[gidx]
        kv = jnp.where(mask, kva[:, :128], 0.0).astype(bf16)
        zm_ref[gidx] = jnp.where(mask, kva[:, 128:], 0.0).astype(bf16)
        m = jnp.dot(kv, wo_v[gidx * 128:(gidx + 1) * 128, :], preferred_element_type=f32)
        m_ref[gidx * 128:(gidx + 1) * 128, :] = m.astype(bf16)

    gwb = jnp.broadcast_to(gw_ref[...], (128, D))

    def q_body(c, carry):
        x = x_v[c]
        gl = jax.lax.dot_general(x, gwb, (((1,), (1,)), ((), ())),
                                 preferred_element_type=f32)
        g = jax.nn.sigmoid(gl)
        g_ref[c] = 1.0 - g
        q = jnp.dot(x, wq_v[...], preferred_element_type=f32)
        pq = _phi(q)
        parts = []
        for j in range(NG):
            pqj = pq[:, j * 128:(j + 1) * 128]
            den = jnp.dot(pqj.astype(bf16), zm_ref[j], preferred_element_type=f32) + 1e-6
            parts.append((pqj * (g / den)).astype(bf16))
        pn = jnp.concatenate(parts, axis=1)
        acc_ref[c] = jnp.dot(pn, m_ref[...], preferred_element_type=f32)
        return carry

    jax.lax.fori_loop(0, NC, q_body, 0)

    def f_body(i, carry):
        c = i // NF
        s = i % NF

        @pl.when(c == 0)
        def _():
            cp_1(s).wait()
            cp_3(s).wait()
            cp_2(s).wait()

        x = x_v[c]
        gate = jnp.dot(x, w1_v[s], preferred_element_type=f32)
        up = jnp.dot(x, w3_v[s], preferred_element_type=f32)
        omg = g_ref[c]
        parts = []
        for j in range(T // 128):
            gj = gate[:, j * 128:(j + 1) * 128]
            uj = up[:, j * 128:(j + 1) * 128]
            parts.append((jax.nn.silu(gj) * uj * omg).astype(bf16))
        h = jnp.concatenate(parts, axis=1)
        acc_ref[c] += jnp.dot(h, w2_v[s], preferred_element_type=f32)

        @pl.when(s == NF - 1)
        def _():
            o_v[c] = acc_ref[c].astype(bf16)
            cp_out(c).start()

        return carry

    jax.lax.fori_loop(0, NC * NF, f_body, 0)

    for c in range(NC):
        cp_out(c).wait()


@jax.jit
def pallas_gated_mix__linear_attn_block__glu_gated_swiglu__prompt_kernel(
    A_x: jax.Array,
    A_wqkv: jax.Array,
    A_wo: jax.Array,
    B_x: jax.Array,
    B_w1: jax.Array,
    B_w3: jax.Array,
    B_w2: jax.Array,
    gate_w: jax.Array,
):
    x = A_x.reshape(S, D)
    gw = gate_w.reshape(1, D)
    any_spec = pl.BlockSpec(memory_space=pl.ANY)
    out = pl.pallas_call(
        _kernel,
        in_specs=[any_spec, pl.BlockSpec(memory_space=pltpu.VMEM),
                  any_spec, any_spec, any_spec, any_spec, any_spec],
        out_specs=any_spec,
        out_shape=jax.ShapeDtypeStruct((S, D), bf16),
        scratch_shapes=[
            pltpu.VMEM((NC, TM, D), bf16),
            pltpu.VMEM((D, D), bf16),
            pltpu.VMEM((NA, D, T), bf16),
            pltpu.VMEM((NA, D, T), bf16),
            pltpu.VMEM((D, D), bf16),
            pltpu.VMEM((NF, D, T), bf16),
            pltpu.VMEM((NF, D, T), bf16),
            pltpu.VMEM((NF, T, D), bf16),
            pltpu.VMEM((NC, TM, D), f32),
            pltpu.VMEM((NG, 128, 256), f32),
            pltpu.VMEM((D, D), bf16),
            pltpu.VMEM((NG, 128, 128), bf16),
            pltpu.VMEM((NC, TM, 128), f32),
            pltpu.VMEM((NC, TM, D), bf16),
            pltpu.SemaphoreType.DMA((NC,)),
            pltpu.SemaphoreType.DMA((1,)),
            pltpu.SemaphoreType.DMA((NA,)),
            pltpu.SemaphoreType.DMA((NA,)),
            pltpu.SemaphoreType.DMA((1,)),
            pltpu.SemaphoreType.DMA((NF,)),
            pltpu.SemaphoreType.DMA((NF,)),
            pltpu.SemaphoreType.DMA((NF,)),
            pltpu.SemaphoreType.DMA((NC,)),
        ],
        compiler_params=pltpu.CompilerParams(
            vmem_limit_bytes=110 * 1024 * 1024,
        ),
    )(x, gw, A_wqkv, A_wo, B_w1, B_w3, B_w2)
    return out.reshape(1, S, D)
```

```python
import jax
import jax.numpy as jnp
import jax.experimental.pallas as pl
import jax.experimental.pallas.tpu as pltpu

S = 2048
D = 1024
F = 3584
DH = 32
TMK = 512
NCK = S // TMK
TK = 512
NA = D // TK
TR = 256
NCR = S // TR
NFD = 2
TFD = F // NFD
NG = D // 128

f32 = jnp.float32
bf16 = jnp.bfloat16


def _phi(t):
    return jnp.where(t > 0, t + 1.0, jnp.exp(t)) + 1e-6


def _blk(i, n):
    return pl.ds(pl.multiple_of(i * n, n), n)


def _kernel(x_hbm, gw_hbm, wqkv_hbm, wo_hbm, w1_hbm, w3_hbm, w2_hbm,
            o_hbm,
            x_v, wq_v, wk_v, wv_v, wo_v, w1_v, w3_v, w2_v,
            gw1_ref, gw_ref, kv_ref, z_ref, m_ref, zm_ref, o_v,
            sem_x, sem_q, sem_k, sem_v, sem_o, sem_1, sem_3, sem_2, sem_out, sem_g):

    def cp_x(c):
        return pltpu.make_async_copy(x_hbm.at[_blk(c, TMK), :], x_v.at[_blk(c, TMK), :], sem_x.at[c])

    def cp_g():
        return pltpu.make_async_copy(gw_hbm, gw1_ref, sem_g.at[0])

    def cp_q():
        return pltpu.make_async_copy(wqkv_hbm.at[:, pl.ds(0, D)], wq_v, sem_q.at[0])

    def cp_k(j):
        return pltpu.make_async_copy(wqkv_hbm.at[:, pl.ds(D + j * TK, TK)], wk_v.at[j], sem_k.at[j])

    def cp_v(j):
        return pltpu.make_async_copy(wqkv_hbm.at[:, pl.ds(2 * D + j * TK, TK)], wv_v.at[j], sem_v.at[j])

    def cp_o():
        return pltpu.make_async_copy(wo_hbm, wo_v, sem_o.at[0])

    def cp_1(j):
        return pltpu.make_async_copy(w1_hbm.at[:, pl.ds(j * TFD, TFD)],
                                     w1_v.at[:, pl.ds(j * TFD, TFD)], sem_1.at[j])

    def cp_3(j):
        return pltpu.make_async_copy(w3_hbm.at[:, pl.ds(j * TFD, TFD)],
                                     w3_v.at[:, pl.ds(j * TFD, TFD)], sem_3.at[j])

    def cp_2(j):
        return pltpu.make_async_copy(w2_hbm.at[pl.ds(j * TFD, TFD), :],
                                     w2_v.at[pl.ds(j * TFD, TFD), :], sem_2.at[j])

    def cp_out(c):
        return pltpu.make_async_copy(o_v.at[_blk(c, TR), :], o_hbm.at[_blk(c, TR), :], sem_out.at[c])

    cp_x(0).start()
    cp_k(0).start()
    cp_v(0).start()
    kv_ref[...] = jnp.zeros_like(kv_ref)
    z_ref[...] = jnp.zeros_like(z_ref)
    cp_x(0).wait()
    cp_k(0).wait()
    cp_v(0).wait()
    for c in range(1, NCK):
        cp_x(c).start()
    for j in range(1, NA):
        cp_k(j).start()
        cp_v(j).start()

    def kv_body(i, carry):
        s = i // NCK
        c = i % NCK

        @pl.when(jnp.logical_and(s == 0, c > 0))
        def _():
            cp_x(c).wait()

        @pl.when(jnp.logical_and(c == 0, s > 0))
        def _():
            cp_k(s).wait()
            cp_v(s).wait()

        @pl.when(i == 1)
        def _():
            cp_g().start()
            cp_o().start()
            cp_q().start()
            for j in range(NFD):
                cp_1(j).start()
                cp_3(j).start()
                cp_2(j).start()

        x = x_v[_blk(c, TMK), :]
        k = jnp.dot(x, wk_v[s], preferred_element_type=f32)
        v = jnp.dot(x, wv_v[s], preferred_element_type=f32)
        pkf = _phi(k)
        pk = pkf.astype(bf16)
        vb = v.astype(bf16)
        z_ref[:, _blk(s, TK)] += jnp.sum(pkf.reshape(TMK // 8, 8, TK), axis=0)
        for j in range(TK // 128):
            kv = jax.lax.dot_general(pk[:, j * 128:(j + 1) * 128], vb[:, j * 128:(j + 1) * 128],
                                     (((0,), (0,)), ((), ())),
                                     preferred_element_type=f32)
            kv_ref[s * (TK // 128) + j] += kv
        return carry

    jax.lax.fori_loop(0, NA * NCK, kv_body, 0)

    cp_g().wait()
    cp_o().wait()
    cp_q().wait()
    for j in range(NFD):
        cp_1(j).wait()
        cp_3(j).wait()
        cp_2(j).wait()
    gw_ref[...] = gw1_ref[...].astype(f32).reshape(1, D)
    ri = jax.lax.broadcasted_iota(jnp.int32, (128, 128), 0) // DH
    ci = jax.lax.broadcasted_iota(jnp.int32, (128, 128), 1) // DH
    mask = ri == ci
    zrow = jnp.sum(z_ref[...], axis=0, keepdims=True)
    for gi in range(NG):
        kv = jnp.where(mask, kv_ref[gi], 0.0).astype(bf16)
        zc = jnp.broadcast_to(zrow[:, gi * 128:(gi + 1) * 128], (128, 128)).T
        zm_ref[gi] = jnp.where(mask, zc, 0.0).astype(bf16)
        m = jnp.dot(kv, wo_v[gi * 128:(gi + 1) * 128, :], preferred_element_type=f32)
        m_ref[gi * 128:(gi + 1) * 128, :] = m.astype(bf16)

    def main_body(c, carry):
        rows = _blk(c, TR)
        x = x_v[rows, :]

        pq = _phi(jnp.dot(x, wq_v[...], preferred_element_type=f32))
        parts = []
        for j in range(NG):
            pqj = pq[:, j * 128:(j + 1) * 128]
            den = jnp.dot(pqj.astype(bf16), zm_ref[j], preferred_element_type=f32) + 1e-6
            r0 = pl.reciprocal(den, approx=True)
            r = r0 * (2.0 - den * r0)
            parts.append((pqj * r).astype(bf16))
        pn = jnp.concatenate(parts, axis=1)
        a = jnp.dot(pn, m_ref[...], preferred_element_type=f32)

        gate = jnp.dot(x, w1_v[...], preferred_element_type=f32)
        up = jnp.dot(x, w3_v[...], preferred_element_type=f32)
        h = (jax.nn.silu(gate) * up).astype(bf16)
        b = jnp.dot(h, w2_v[...], preferred_element_type=f32)

        gl = jnp.sum(x.astype(f32) * gw_ref[...], axis=-1, keepdims=True)
        g = jax.nn.sigmoid(gl)
        o_v[rows, :] = (b + g * (a - b)).astype(bf16)
        cp_out(c).start()
        return carry

    jax.lax.fori_loop(0, NCR, main_body, 0)

    for c in range(NCR):
        cp_out(c).wait()


@jax.jit
def pallas_gated_mix__linear_attn_block__glu_gated_swiglu__prompt_kernel(
    A_x: jax.Array,
    A_wqkv: jax.Array,
    A_wo: jax.Array,
    B_x: jax.Array,
    B_w1: jax.Array,
    B_w3: jax.Array,
    B_w2: jax.Array,
    gate_w: jax.Array,
):
    x = A_x.reshape(S, D)
    any_spec = pl.BlockSpec(memory_space=pl.ANY)
    out = pl.pallas_call(
        _kernel,
        in_specs=[any_spec] * 7,
        out_specs=any_spec,
        out_shape=jax.ShapeDtypeStruct((S, D), bf16),
        scratch_shapes=[
            pltpu.VMEM((S, D), bf16),
            pltpu.VMEM((D, D), bf16),
            pltpu.VMEM((NA, D, TK), bf16),
            pltpu.VMEM((NA, D, TK), bf16),
            pltpu.VMEM((D, D), bf16),
            pltpu.VMEM((D, F), bf16),
            pltpu.VMEM((D, F), bf16),
            pltpu.VMEM((F, D), bf16),
            pltpu.VMEM((D,), bf16),
            pltpu.VMEM((1, D), f32),
            pltpu.VMEM((NG, 128, 128), f32),
            pltpu.VMEM((8, D), f32),
            pltpu.VMEM((D, D), bf16),
            pltpu.VMEM((NG, 128, 128), bf16),
            pltpu.VMEM((S, D), bf16),
            pltpu.SemaphoreType.DMA((NCK,)),
            pltpu.SemaphoreType.DMA((1,)),
            pltpu.SemaphoreType.DMA((NA,)),
            pltpu.SemaphoreType.DMA((NA,)),
            pltpu.SemaphoreType.DMA((1,)),
            pltpu.SemaphoreType.DMA((NFD,)),
            pltpu.SemaphoreType.DMA((NFD,)),
            pltpu.SemaphoreType.DMA((NFD,)),
            pltpu.SemaphoreType.DMA((NCR,)),
            pltpu.SemaphoreType.DMA((1,)),
        ],
        compiler_params=pltpu.CompilerParams(
            vmem_limit_bytes=110 * 1024 * 1024,
        ),
    )(x, gate_w, A_wqkv, A_wo, B_w1, B_w3, B_w2)
    return out.reshape(1, S, D)
```
